```python
import jax
import jax.numpy as jnp

def _softmax(x, axis=-1):
    return jax.nn.softmax(x, axis=axis)
def _gelu(x):
    return jax.nn.gelu(x, approximate=True)
def _silu(x):
    return jax.nn.silu(x)
def _sigmoid(x):
    return jax.nn.sigmoid(x)
def _layernorm(x, axis=-1, eps=1e-5):
    m = jnp.mean(x, axis=axis, keepdims=True)
    v = jnp.var(x, axis=axis, keepdims=True)
    return (x - m) / jnp.sqrt(v + eps)
def _scatter_add(tgt, idx, src, axis=0):
    return tgt.at[idx].add(src)
def _segment_sum(src, seg, n):
    return jax.ops.segment_sum(src, seg, n)
class _Rng:
    def __init__(self, key):
        self._k = key
    def _next(self):
        self._k, sub = jax.random.split(self._k)
        return sub
    def normal(self, shape):
        return jax.random.normal(self._next(), shape, dtype=jnp.bfloat16)
    def randint(self, lo, hi, shape):
        return jax.random.randint(self._next(), shape, lo, hi, dtype=jnp.int32)
    def uniform(self, shape, lo=0.0, hi=1.0):
        return jax.random.uniform(self._next(), shape, jnp.bfloat16, lo, hi)
    def permutation(self, n):
        return jax.random.permutation(self._next(), n)


kernel_name = 'standalone__modern_conv_block_replknet__vision'

def setup_inputs():
    _rng = _Rng(jax.random.key(int.from_bytes(__import__("os").urandom(4), "little")))
    _w = (lambda a: (lambda t: t.astype(jnp.bfloat16) if jnp.issubdtype(t.dtype, jnp.floating) else t)(jnp.asarray(a)))
    H = W = 512
    C = 96
    K = 3
    return {
        "x": _w((lambda *s: _rng.normal(s) * 0.05)(1, H, W, C)),
        "dw_large": _w((lambda *s: _rng.normal(s) * 0.05)(K, K, C) * (1.0 / K)),
        "dw_small": _w((lambda *s: _rng.normal(s) * 0.05)(5, 5, C) * 0.2),
        "w1": _w((lambda *s: _rng.normal(s) * 0.05)(C, 4 * C) * (C ** -0.5)),
        "w2": _w((lambda *s: _rng.normal(s) * 0.05)(4 * C, C) * ((4 * C) ** -0.5)),
    }

def reference(x, dw_large, dw_small, w1, w2):
    B, H, W, C = x.shape
    Kl = dw_large.shape[0]
    pl = (Kl - 1) // 2
    xpl = jnp.pad(x, ((0,0),(pl,pl),(pl,pl),(0,0)))
    out = jnp.zeros_like(x)
    for i in range(Kl):
        for j in range(Kl):
            out = out + xpl[:, i:i+H, j:j+W, :] * dw_large[i, j][None, None, None, :]
    Ks = dw_small.shape[0]
    ps = (Ks - 1) // 2
    xps = jnp.pad(x, ((0,0),(ps,ps),(ps,ps),(0,0)))
    for i in range(Ks):
        for j in range(Ks):
            out = out + xps[:, i:i+H, j:j+W, :] * dw_small[i, j][None, None, None, :]
    h = _layernorm(out, axis=-1)
    h = _gelu(jnp.einsum('bhwc,ce->bhwe', h, w1))
    h = jnp.einsum('bhwe,ec->bhwc', h, w2)
    return x + h
```

```python
import functools
import math

import jax
import jax.numpy as jnp
import jax.experimental.pallas as pl
import jax.experimental.pallas.tpu as pltpu

HB = 32


def _kernel(x_ref, top_ref, bot_ref, dwl_ref, dws_ref, w1_ref, w2_ref, o_ref,
            kb_ref, w1t_ref, w2t_ref, xf_ref, n_ref, *, hb, nblk):
    _, C, W = x_ref.shape
    step = pl.program_id(0)
    f32 = jnp.float32

    @pl.when(step == 0)
    def _():
        for i in range(5):
            for j in range(5):
                k = dws_ref[i, j:j + 1, :].astype(f32)
                if 1 <= i <= 3 and 1 <= j <= 3:
                    k = k + dwl_ref[i - 1, j - 1:j, :].astype(f32)
                k = jnp.concatenate([k, jnp.zeros((1, 128 - C), f32)], axis=1)
                kt = jnp.broadcast_to(k, (128, 128)).T
                kb_ref[i * 5 + j] = kt[:C, :]
        w1 = jnp.concatenate(
            [w1_ref[...].astype(f32), jnp.zeros((128 - C, 4 * C), f32)], axis=0)
        w1t_ref[...] = w1.T[:, :C].astype(jnp.bfloat16)
        w2 = jnp.concatenate(
            [w2_ref[...].astype(f32), jnp.zeros((4 * C, 128 - C), f32)], axis=1)
        w2t_ref[...] = (0.5 * w2.T[:C, :]).astype(jnp.bfloat16)

    zero2 = jnp.zeros((2, C, W), f32)
    xf_ref[0:2] = jnp.where(step > 0, top_ref[...].astype(f32), zero2)
    xf_ref[hb + 2:hb + 4] = jnp.where(step < nblk - 1, bot_ref[...].astype(f32), zero2)
    xf_ref[2:4] = x_ref[0:2].astype(f32)

    lane = jax.lax.broadcasted_iota(jnp.int32, (8, W), 1)

    def conv_ln(r):
        outs = []
        for g in range(C // 8):
            cs = slice(g * 8, g * 8 + 8)
            xs = [xf_ref[r + i, cs, :] for i in range(5)]
            acc = None
            for j in (2, 0, 1, 3, 4):
                y = None
                for i in range(5):
                    k = kb_ref[i * 5 + j, cs, :]
                    k = jnp.concatenate([k] * (W // 128), axis=1)
                    t = xs[i] * k
                    y = t if y is None else y + t
                s = j - 2
                if s != 0:
                    y = pltpu.roll(y, (-s) % W, axis=1)
                    parts = [y[:, t * 128:(t + 1) * 128] for t in range(W // 128)]
                    l = lane[:, :128]
                    if s > 0:
                        parts[-1] = jnp.where(l < 128 - s, parts[-1], 0.0)
                    else:
                        parts[0] = jnp.where(l >= -s, parts[0], 0.0)
                    y = jnp.concatenate(parts, axis=1)
                acc = y if acc is None else acc + y
            outs.append(acc)
        o = jnp.concatenate(outs, axis=0)
        m = jnp.mean(o, axis=0, keepdims=True)
        d = o - m
        v = jnp.mean(d * d, axis=0, keepdims=True)
        return (d * jax.lax.rsqrt(v + 1e-5)).astype(jnp.bfloat16)

    c0 = math.sqrt(2.0 / math.pi)
    c1 = c0 * 0.044715

    def mlp(r, n):
        h = jnp.dot(w1t_ref[...], n, preferred_element_type=f32)
        u = h * (h * h * c1 + c0)
        g = (h + h * jnp.tanh(u)).astype(jnp.bfloat16)
        y = jnp.dot(w2t_ref[...], g, preferred_element_type=f32)
        o_ref[r] = (xf_ref[r + 2] + y).astype(o_ref.dtype)

    n_ref[...] = conv_ln(0)

    def body(r, carry):
        @pl.when(r + 3 < hb)
        def _():
            xf_ref[r + 5] = x_ref[jnp.minimum(r + 3, hb - 1)].astype(f32)
        mlp(r, n_ref[...])
        n_ref[...] = conv_ln(r + 1)
        return carry

    xf_ref[4] = x_ref[2].astype(f32)
    jax.lax.fori_loop(0, hb - 1, body, 0)
    mlp(hb - 1, n_ref[...])


@jax.jit
def pallas_standalone__modern_conv_block_replknet__vision_kernel(
    x: jax.Array,
    dw_large: jax.Array,
    dw_small: jax.Array,
    w1: jax.Array,
    w2: jax.Array,
):
    B, H, W, C = x.shape
    hb = HB
    nblk = H // hb
    xt = jnp.transpose(x, (0, 1, 3, 2)).reshape(H, C, W)
    full = lambda a: pl.BlockSpec(a.shape, lambda i: (0,) * a.ndim)
    out = pl.pallas_call(
        functools.partial(_kernel, hb=hb, nblk=nblk),
        grid=(nblk,),
        in_specs=[
            pl.BlockSpec((hb, C, W), lambda i: (i, 0, 0)),
            pl.BlockSpec((2, C, W), lambda i: (jnp.maximum(i * (hb // 2) - 1, 0), 0, 0)),
            pl.BlockSpec((2, C, W), lambda i: (jnp.minimum((i + 1) * (hb // 2), H // 2 - 1), 0, 0)),
            full(dw_large), full(dw_small), full(w1), full(w2),
        ],
        out_specs=pl.BlockSpec((hb, C, W), lambda i: (i, 0, 0)),
        out_shape=jax.ShapeDtypeStruct((H, C, W), x.dtype),
        scratch_shapes=[
            pltpu.VMEM((25, C, 128), jnp.float32),
            pltpu.VMEM((4 * C, C), jnp.bfloat16),
            pltpu.VMEM((C, 4 * C), jnp.bfloat16),
            pltpu.VMEM((hb + 4, C, W), jnp.float32),
            pltpu.VMEM((C, W), jnp.bfloat16),
        ],
        compiler_params=pltpu.CompilerParams(
            dimension_semantics=("arbitrary",),
            vmem_limit_bytes=100 * 1024 * 1024,
        ),
    )(xt, xt, xt, dw_large, dw_small, w1, w2)
    return jnp.transpose(out.reshape(B, H, C, W), (0, 1, 3, 2))
```

```python
import functools
import math

import jax
import jax.numpy as jnp
import jax.experimental.pallas as pl
import jax.experimental.pallas.tpu as pltpu

HB = 8


def _kernel(x_ref, dwl_ref, dws_ref, w1_ref, w2_ref, o_ref,
            kb_ref, w1t_ref, w2t_ref, xf_ref, n_ref, g_ref, *, hb, nblk):
    _, C, W = x_ref.shape
    step = pl.program_id(0)
    f32 = jnp.float32

    @pl.when(step == 0)
    def _():
        for i in range(5):
            for j in range(5):
                k = dws_ref[i, j:j + 1, :].astype(f32)
                if 1 <= i <= 3 and 1 <= j <= 3:
                    k = k + dwl_ref[i - 1, j - 1:j, :].astype(f32)
                k = jnp.concatenate([k, jnp.zeros((1, 128 - C), f32)], axis=1)
                kt = jnp.broadcast_to(k, (128, 128)).T
                kb_ref[i * 5 + j] = kt[:C, :]
        w1 = jnp.concatenate(
            [w1_ref[...].astype(f32), jnp.zeros((128 - C, 4 * C), f32)], axis=0)
        w1t_ref[...] = w1.T[:, :C].astype(jnp.bfloat16)
        w2 = jnp.concatenate(
            [w2_ref[...].astype(f32), jnp.zeros((4 * C, 128 - C), f32)], axis=1)
        w2t_ref[...] = (0.5 * w2.T[:C, :]).astype(jnp.bfloat16)

        xf_ref[...] = jnp.zeros(xf_ref.shape, f32)
        n_ref[...] = jnp.zeros(n_ref.shape, n_ref.dtype)
        g_ref[...] = jnp.zeros(g_ref.shape, g_ref.dtype)

    new = (step % 2) * hb
    old = hb - new

    @pl.when(step == nblk)
    def _():
        xf_ref[pl.ds(new, hb)] = jnp.zeros((hb, C, W), f32)

    lane = jax.lax.broadcasted_iota(jnp.int32, (8, W), 1)

    def conv_ln(r):
        outs = []
        for g in range(C // 8):
            cs = slice(g * 8, g * 8 + 8)
            xs = [xf_ref[(old + r + i) % (2 * hb), cs, :] for i in range(5)]
            acc = None
            for j in (2, 0, 1, 3, 4):
                y = None
                for i in range(5):
                    k = kb_ref[i * 5 + j, cs, :]
                    k = jnp.concatenate([k] * (W // 128), axis=1)
                    t = xs[i] * k
                    y = t if y is None else y + t
                s = j - 2
                if s != 0:
                    y = pltpu.roll(y, (-s) % W, axis=1)
                    parts = [y[:, t * 128:(t + 1) * 128] for t in range(W // 128)]
                    l = lane[:, :128]
                    if s > 0:
                        parts[-1] = jnp.where(l < 128 - s, parts[-1], 0.0)
                    else:
                        parts[0] = jnp.where(l >= -s, parts[0], 0.0)
                    y = jnp.concatenate(parts, axis=1)
                acc = y if acc is None else acc + y
            outs.append(acc)
        o = jnp.concatenate(outs, axis=0)
        m = jnp.mean(o, axis=0, keepdims=True)
        d = o - m
        v = jnp.mean(d * d, axis=0, keepdims=True)
        return (d * jax.lax.rsqrt(v + 1e-5)).astype(jnp.bfloat16)

    c0 = math.sqrt(2.0 / math.pi)
    c1 = c0 * 0.044715

    def body(r, carry):
        y = jnp.dot(w2t_ref[...], g_ref[...], preferred_element_type=f32)
        o_ref[r] = (xf_ref[old + r] + y).astype(o_ref.dtype)
        h = jnp.dot(w1t_ref[...], n_ref[...], preferred_element_type=f32)
        u = h * (h * h * c1 + c0)
        g_ref[...] = (h + h * jnp.tanh(u)).astype(jnp.bfloat16)
        n_ref[...] = conv_ln(r)
        xf_ref[jnp.where(step < nblk, new + r, 2 * hb)] = x_ref[r].astype(f32)
        return carry

    jax.lax.fori_loop(0, hb, body, 0)


@jax.jit
def pallas_standalone__modern_conv_block_replknet__vision_kernel(
    x: jax.Array,
    dw_large: jax.Array,
    dw_small: jax.Array,
    w1: jax.Array,
    w2: jax.Array,
):
    B, H, W, C = x.shape
    hb = HB
    nblk = H // hb
    xt = jnp.transpose(x, (0, 1, 3, 2)).reshape(H, C, W)
    full = lambda a: pl.BlockSpec(a.shape, lambda i: (0,) * a.ndim)
    out = pl.pallas_call(
        functools.partial(_kernel, hb=hb, nblk=nblk),
        grid=(nblk + 1,),
        in_specs=[
            pl.BlockSpec((hb, C, W), lambda i: (jnp.minimum(i, nblk - 1), 0, 0)),
            full(dw_large), full(dw_small), full(w1), full(w2),
        ],
        out_specs=pl.BlockSpec((hb, C, W), lambda i: (jnp.maximum(i - 1, 0), 0, 0)),
        out_shape=jax.ShapeDtypeStruct((H, C, W), x.dtype),
        scratch_shapes=[
            pltpu.VMEM((25, C, 128), jnp.float32),
            pltpu.VMEM((4 * C, C), jnp.bfloat16),
            pltpu.VMEM((C, 4 * C), jnp.bfloat16),
            pltpu.VMEM((2 * hb + 1, C, W), jnp.float32),
            pltpu.VMEM((C, W), jnp.bfloat16),
            pltpu.VMEM((4 * C, W), jnp.bfloat16),
        ],
        compiler_params=pltpu.CompilerParams(
            dimension_semantics=("arbitrary",),
            vmem_limit_bytes=100 * 1024 * 1024,
            flags={"XLA_TPU_FORCE_LP_LLO_SCHEDULER": True},
        ),
    )(xt, dw_large, dw_small, w1, w2)
    return jnp.transpose(out.reshape(B, H, C, W), (0, 1, 3, 2))
```
